```python
import os as _os
_os.environ.setdefault("JAX_PLATFORMS", "cpu")
import jax
import jax.numpy as jnp

def _softmax(x, axis=-1):
    return jax.nn.softmax(x, axis=axis)
def _gelu(x):
    return jax.nn.gelu(x, approximate=True)
def _silu(x):
    return jax.nn.silu(x)
def _sigmoid(x):
    return jax.nn.sigmoid(x)
def _layernorm(x, axis=-1, eps=1e-5):
    m = jnp.mean(x, axis=axis, keepdims=True)
    v = jnp.var(x, axis=axis, keepdims=True)
    return (x - m) / jnp.sqrt(v + eps)
def _scatter_add(tgt, idx, src, axis=0):
    return tgt.at[idx].add(src)
def _segment_sum(src, seg, n):
    return jax.ops.segment_sum(src, seg, n)
class _Rng:
    def __init__(self, key):
        self._k = key
    def _next(self):
        self._k, sub = jax.random.split(self._k)
        return sub
    def normal(self, shape):
        return jax.random.normal(self._next(), shape, dtype=jnp.bfloat16)
    def randint(self, lo, hi, shape):
        return jax.random.randint(self._next(), shape, lo, hi, dtype=jnp.int32)
    def uniform(self, shape, lo=0.0, hi=1.0):
        return jax.random.uniform(self._next(), shape, jnp.bfloat16, lo, hi)
    def permutation(self, n):
        return jax.random.permutation(self._next(), n)


kernel_name = 'gated_mix__mha_block__ssm_conv_h3__prompt'

def setup_inputs():
    _rng = _Rng(jax.random.key(int.from_bytes(__import__("os").urandom(4), "little")))
    _w = (lambda a: (lambda t: t.astype(jnp.bfloat16) if jnp.issubdtype(t.dtype, jnp.floating) else t)(jnp.asarray(a)))
    def _A_setup():
        B, S, D, H = 1, 2048, 640, 32
        return {
            "x": _w((lambda *s: _rng.normal(s) * 0.05)(B, S, D)),
            "wqkv": _w((lambda *s: _rng.normal(s) * 0.4)(D, 3 * D)),
            "wo": _w((lambda *s: _rng.normal(s) * 0.05)(D, D)),
        }
    _A_in = _A_setup()

    def _B_setup():
        B, S, D = 1, 2048, 640
        ks = 4
        return {
            "q": _w((lambda *s: _rng.normal(s) * 0.05)(B, S, D)),
            "k": _w((lambda *s: _rng.normal(s) * 0.4)(B, S, D)),
            "v": _w((lambda *s: _rng.normal(s) * 0.4)(B, S, D)),
            "shift_k": _w((lambda *s: _rng.normal(s) * 0.4)(D, ks) * 0.5),
            "ssm_k": _w((lambda *s: _rng.normal(s) * 0.4)(D, S) * (1.0 / S ** 0.5)),
            "ssm_D": _w((lambda *s: _rng.normal(s) * 0.4)(D)),
        }
    _B_in = _B_setup()

    return {
        "A_x": _A_in["x"],
        "A_wqkv": _A_in["wqkv"],
        "A_wo": _A_in["wo"],
        "B_q": _B_in["q"],
        "B_k": _B_in["k"],
        "B_v": _B_in["v"],
        "B_shift_k": _B_in["shift_k"],
        "B_ssm_k": _B_in["ssm_k"],
        "B_ssm_D": _B_in["ssm_D"],
        "gate_w": _w((lambda *s: _rng.normal(s) * 0.05)(640) * 16.0),
    }

def reference(A_x, A_wqkv, A_wo, B_q, B_k, B_v, B_shift_k, B_ssm_k, B_ssm_D, gate_w):
    def _A_ref(x, wqkv, wo):
        B, S, D = x.shape
        H = 32
        Dh = D // H
        qkv = (lambda x, *d: x.transpose(*d))((x @ wqkv).reshape(B, S, 3, H, Dh), 2, 0, 3, 1, 4)
        q, k, v = qkv[0], qkv[1], qkv[2]
        scores = jnp.einsum("bhqd,bhkd->bhqk", q, k) * (Dh ** -0.5)
        p = _softmax(scores, axis=-1)
        o = jnp.einsum("bhqk,bhkd->bhqd", p, v)
        return (lambda x, *d: x.transpose(*d))(o, 0, 2, 1, 3).reshape(B, S, D) @ wo

    def _B_ref(q, k, v, shift_k, ssm_k, ssm_D):
        B, S, D = q.shape
        ks = shift_k.shape[-1]
        k_pad = jnp.pad(k, ((0, 0), (ks - 1, 0), (0, 0)))
        k_shift = jnp.zeros_like(k)
        for t in range(ks):
            k_shift = k_shift + k_pad[:, t:t + S, :] * shift_k[:, ks - 1 - t][None, None, :]
        kv = k_shift * v
        L = 2 * S
        kv_pad = jnp.pad(kv, ((0, 0), (0, S), (0, 0)))
        kf_pad = jnp.pad(ssm_k, ((0, 0), (0, S)))
        kv_f = (lambda x, axes=(-2,-1): jnp.fft.rfft2(x.astype(jnp.float32), axes=axes))(kv_pad[:, None, :, :], axes=(1, 2))
        kf_f = (lambda x, axes=(-2,-1): jnp.fft.rfft2(x.astype(jnp.float32), axes=axes))(kf_pad[:, None, :], axes=(1, 2))
        kf_f = (lambda x, *d: x.transpose(*d))(kf_f, 1, 2, 0)
        y_f = kv_f * kf_f[None, :, :, :]
        y = (lambda x, s, axes=(-2,-1): jnp.fft.irfft2(x, s=s, axes=axes).astype(jnp.bfloat16))(y_f, (1, L), axes=(1, 2))[:, 0, :S, :]
        y = y + kv * ssm_D[None, None, :]
        return q * y

    x = A_x
    g = _sigmoid((x * gate_w).sum(-1, keepdims=True))
    a = _A_ref(x, A_wqkv, A_wo)
    b = _B_ref(x, B_k, B_v, B_shift_k, B_ssm_k, B_ssm_D)
    return g * a + (1 - g) * b
```

```python
import numpy as np

import jax
import jax.numpy as jnp
from jax import lax
import jax.experimental.pallas as pl
import jax.experimental.pallas.tpu as pltpu

S = 2048
D = 640
H = 32
DH = D // H
NB = D // 128
L = 128
NC = S // L
TQ = 512
KC = 128
RB = 256

BF = jnp.bfloat16
F32 = jnp.float32
I32 = jnp.int32

QSCALE = float(DH ** -0.5 * np.log2(np.e))
L_MIN = float(2.0 ** -40)
L_MAX = float(2.0 ** 60)


def _dft_tables():
    f = np.concatenate([np.arange(0, L, 2), np.arange(1, L, 2)]).astype(np.float64)
    n = np.arange(L, dtype=np.float64)
    ang = np.pi * (f[:, None] + 0.5) * n[None, :] / L
    fwd = np.concatenate([np.cos(ang), -np.sin(ang)], axis=0)
    inv = fwd.T / L
    return fwd.astype(BF), inv.astype(BF)


def _dot(a, b, ca=1, cb=0):
    return lax.dot_general(a, b, (((ca,), (cb,)), ((), ())), preferred_element_type=F32)


def _kernel(x_hbm, w_hbm, wo_hbm, k_hbm, v_hbm, sh_ref, sk_hbm, sd_ref, gw_ref, fwd_ref, inv_ref,
            out_hbm,
            x_v, w_v, wo_v, k_v, v_v, sk_v, par_v, kpad, kv_v, uf, kf, yf, b_v, g_v,
            qt_v, vt_v, kk_v, ot_v, out_v, sems, osems):
    def col(ref, c):
        return ref.at[:, pl.ds(pl.multiple_of(c * 128, 128), 128)]

    def blk_copies(i):
        cps = [pltpu.make_async_copy(col(w_hbm, t * NB + i), w_v.at[i, t], sems.at[i, t]) for t in range(3)]
        cps.append(pltpu.make_async_copy(col(k_hbm, i), k_v.at[i], sems.at[i, 3]))
        cps.append(pltpu.make_async_copy(col(v_hbm, i), v_v.at[i], sems.at[i, 4]))
        cps.append(pltpu.make_async_copy(
            sk_hbm.at[pl.ds(pl.multiple_of(i * 128, 128), 128), :], sk_v.at[i], sems.at[i, 5]))
        return cps

    x_cps = [pltpu.make_async_copy(col(x_hbm, i), x_v.at[i], sems.at[i, 6]) for i in range(NB)]
    wo_cp = pltpu.make_async_copy(wo_hbm, wo_v, sems.at[0, 7])
    for cp in x_cps:
        cp.start()
    for i in range(NB):
        for cp in blk_copies(i):
            cp.start()
    wo_cp.start()

    sh = sh_ref[...].astype(F32)
    sd = sd_ref[...].astype(F32).reshape(1, D)
    gw = gw_ref[...].astype(F32).reshape(1, D)
    for i in range(NB):
        cs = slice(i * 128, (i + 1) * 128)
        for j in range(4):
            par_v[i, j] = jnp.broadcast_to(sh[j:j + 1, cs], (8, 128))
        par_v[i, 4] = jnp.broadcast_to(sd[:, cs], (8, 128))
        par_v[i, 5] = jnp.broadcast_to(gw[:, cs], (8, 128))
    kpad[0:8, :] = jnp.zeros((8, 128), F32)
    g_v[...] = jnp.zeros((S, 128), F32)
    for cp in x_cps:
        cp.wait()

    def proj_conv(i, carry):
        for cp in blk_copies(i):
            cp.wait()
        r0 = pl.multiple_of(i * 128, 128)
        wqv = jnp.concatenate([w_v[i, 0].T, w_v[i, 2].T], axis=0)
        wk = w_v[i, 1]

        kpad[8:, :] = k_v[i].astype(F32)
        for c in range(NC):
            acc = None
            for j in range(4):
                t = kpad[8 + c * L - j:8 + (c + 1) * L - j, :] * jnp.tile(par_v[i, j], (L // 8, 1))
                acc = t if acc is None else acc + t
            kv_v[c * L:(c + 1) * L, :] = acc * v_v[i, c * L:(c + 1) * L, :].astype(F32)

        fwd = fwd_ref[...]
        for c in range(0, NC, 4):
            kc = jnp.concatenate([sk_v[i, :, (c + t) * L:(c + t + 1) * L] for t in range(4)], axis=0)
            r = _dot(fwd, kc, 1, 1)
            for t in range(4):
                kf[c + t] = r[:, t * 128:(t + 1) * 128]
        for c in range(0, NC, 4):
            uc = jnp.concatenate([kv_v[(c + t) * L:(c + t + 1) * L, :].astype(BF) for t in range(4)], axis=1)
            r = _dot(fwd, uc)
            for t in range(4):
                uf[c + t] = r[:, t * 128:(t + 1) * 128]

        for r in range(S // 512):
            rs = slice(r * 512, (r + 1) * 512)
            xb = jnp.concatenate([x_v[t, rs, :] for t in range(NB)], axis=1)
            qv = _dot(wqv, xb, 1, 1)
            qt_v[pl.ds(r0, 128), rs] = (qv[:128] * QSCALE).astype(BF).astype(F32)
            vt_v[pl.ds(r0, 128), rs] = qv[128:].astype(BF).astype(F32)
            kk_v[i, r * 256:(r + 1) * 256, :] = pltpu.bitcast(_dot(xb, wk).astype(BF), I32)

        for g in range(L // 8):
            re = slice(g * 8, (g + 1) * 8)
            im = slice(L + g * 8, L + (g + 1) * 8)
            kr, ki = [], []
            for d in range(NC):
                a, b = kf[d, re, :], kf[d, im, :]
                if d > 0:
                    pa, pb = kf[d - 1, re, :], kf[d - 1, im, :]
                    a, b = (a - pb, b + pa) if g < L // 16 else (a + pb, b - pa)
                kr.append(a)
                ki.append(b)
            for o in range(NC):
                yr = yi = None
                for j in range(o + 1):
                    ur, ui = uf[j, re, :], uf[j, im, :]
                    tr = kr[o - j] * ur - ki[o - j] * ui
                    ti = kr[o - j] * ui + ki[o - j] * ur
                    yr, yi = (tr, ti) if yr is None else (yr + tr, yi + ti)
                yf[o, re, :] = yr
                yf[o, im, :] = yi

        inv = inv_ref[...]
        for c in range(0, NC, 4):
            y = _dot(inv, jnp.concatenate([yf[c + t].astype(BF) for t in range(4)], axis=1))
            for t in range(4):
                cs = slice((c + t) * L, (c + t + 1) * L)
                xc = x_v[i, cs, :].astype(F32)
                yy = y[:, t * 128:(t + 1) * 128] + kv_v[cs, :] * jnp.tile(par_v[i, 4], (L // 8, 1))
                b_v[i, cs, :] = xc * yy
                g_v[cs, :] += xc * jnp.tile(par_v[i, 5], (L // 8, 1))
        return carry

    lax.fori_loop(0, NB, proj_conv, 0)

    row24 = lax.broadcasted_iota(I32, (24, 128), 0)
    lane = lax.broadcasted_iota(I32, (8, 128), 1)

    def head_views(h):
        odd = h & 1
        r0 = pl.multiple_of(h * DH - 4 * odd, 8)
        own = (row24 >= 4 * odd) & (row24 < 4 * odd + DH)
        b0 = r0 // 128
        b1 = jnp.minimum(b0 + 1, NB - 1)
        l0 = r0 - b0 * 128
        shift = (128 - l0) & 127

        def keys(a, n):
            m = jnp.tile(lane >= l0, (n // 16, 1))
            rs = pl.ds(a // 2, n // 2)
            kk = jnp.where(m, kk_v[b0, rs, :], kk_v[b1, rs, :])
            return pltpu.bitcast(pltpu.roll(kk, shift, 1), BF)[:, :32]

        def queries(cs, n):
            q = jnp.where(jnp.tile(own, (1, n // 128)), qt_v[pl.ds(r0, 24), cs], 0.0)
            return jnp.concatenate([q, jnp.zeros((8, n), F32)], axis=0).astype(BF)

        def values(cs, n):
            return jnp.where(jnp.tile(own, (1, n // 128)), vt_v[pl.ds(r0, 24), cs], 1.0)

        def denom(o):
            return jnp.where(odd == 1, o[0:1], o[23:24])

        return keys, queries, values, denom

    def head_fast(h, carry):
        lo, hi = carry
        keys, queries, values, denom = head_views(h)
        nq, nk = S // TQ, S // KC
        qs = [queries(slice(j * TQ, (j + 1) * TQ), TQ) for j in range(nq)]
        steps = [(c, j) for c in range(nk) for j in range(nq)]
        lag = 2
        ps, acc, kc, vc = {}, {}, {}, {}
        for t in range(len(steps) + lag):
            if t < len(steps):
                c, j = steps[t]
                if j == 0:
                    kc[c] = keys(c * KC, KC)
                ps[t] = jnp.exp2(_dot(kc[c], qs[j])).astype(BF)
            if t >= lag:
                c, j = steps[t - lag]
                if j == 0:
                    vc[c] = values(slice(c * KC, (c + 1) * KC), KC)
                r = _dot(vc[c], ps.pop(t - lag))
                acc[j] = r if c == 0 else acc[j] + r
                if c == nk - 1:
                    o = acc.pop(j)
                    l = denom(o)
                    ot_v[h, :, j * TQ:(j + 1) * TQ] = o * (1.0 / l)
                    lo = jnp.minimum(lo, l)
                    a = jnp.abs(o)
                    hi = jnp.maximum(hi, jnp.maximum(jnp.maximum(a[0:8], a[8:16]), a[16:24]))
        return lo, hi

    lo, hi = lax.fori_loop(0, H, head_fast, (jnp.ones((1, TQ), F32), jnp.ones((8, TQ), F32)))

    safe = (lo >= L_MIN) & (hi <= L_MAX)
    n_bad = jnp.sum(jnp.where(safe, 0.0, 1.0))

    @pl.when(n_bad > 0.0)
    def _():
        def head_exact(t, carry):
            h = t // (S // 128)
            cs = pl.ds(pl.multiple_of((t % (S // 128)) * 128, 128), 128)
            keys, queries, values, denom = head_views(h)
            s = _dot(keys(0, S), queries(cs, 128))
            p = jnp.exp2(s - jnp.max(s, axis=0, keepdims=True)).astype(BF)
            o = _dot(values(slice(None), S), p)
            ot_v[h, :, cs] = o * (1.0 / denom(o))
            return carry

        lax.fori_loop(0, H * (S // 128), head_exact, 0)

    wo_cp.wait()
    low4 = lax.broadcasted_iota(I32, (8, RB), 0) < 4

    def out_copy(r):
        rs = pl.ds(pl.multiple_of(r * RB, RB), RB)
        return pltpu.make_async_copy(out_v.at[rs, :], out_hbm.at[rs, :], osems.at[r])

    def out_block(r, carry):
        rs = pl.ds(pl.multiple_of(r * RB, RB), RB)
        parts = []
        for p in range(H // 2):
            e, o = ot_v[2 * p, :, rs], ot_v[2 * p + 1, :, rs]
            parts += [e[0:16], jnp.where(low4, e[16:24], o[0:8]), o[8:24]]
        a = _dot(jnp.concatenate(parts, axis=0).astype(BF), wo_v[...], 0, 0)
        g = jax.nn.sigmoid(jnp.sum(g_v[rs, :], axis=1, keepdims=True))
        b = jnp.concatenate([b_v[t, rs, :] for t in range(NB)], axis=1)
        out_v[rs, :] = (g * a + (1.0 - g) * b).astype(BF)
        out_copy(r).start()
        return carry

    lax.fori_loop(0, S // RB, out_block, 0)
    for r in range(S // RB):
        out_copy(r).wait()


@jax.jit
def pallas_gated_mix__mha_block__ssm_conv_h3__prompt_kernel(
    A_x: jax.Array,
    A_wqkv: jax.Array,
    A_wo: jax.Array,
    B_q: jax.Array,
    B_k: jax.Array,
    B_v: jax.Array,
    B_shift_k: jax.Array,
    B_ssm_k: jax.Array,
    B_ssm_D: jax.Array,
    gate_w: jax.Array,
):
    del B_q
    fwd, inv = _dft_tables()
    hbm = pl.BlockSpec(memory_space=pl.ANY)
    vmem = pl.BlockSpec(memory_space=pltpu.VMEM)
    out = pl.pallas_call(
        _kernel,
        in_specs=[hbm, hbm, hbm, hbm, hbm, vmem, hbm, vmem, vmem, vmem, vmem],
        out_specs=hbm,
        out_shape=jax.ShapeDtypeStruct((S, D), BF),
        scratch_shapes=[
            pltpu.VMEM((NB, S, 128), BF),
            pltpu.VMEM((NB, 3, D, 128), BF),
            pltpu.VMEM((D, D), BF),
            pltpu.VMEM((NB, S, 128), BF),
            pltpu.VMEM((NB, S, 128), BF),
            pltpu.VMEM((NB, 128, S), BF),
            pltpu.VMEM((NB, 6, 8, 128), F32),
            pltpu.VMEM((S + 8, 128), F32),
            pltpu.VMEM((S, 128), F32),
            pltpu.VMEM((NC, 2 * L, 128), F32),
            pltpu.VMEM((NC, 2 * L, 128), F32),
            pltpu.VMEM((NC, 2 * L, 128), F32),
            pltpu.VMEM((NB, S, 128), F32),
            pltpu.VMEM((S, 128), F32),
            pltpu.VMEM((D, S), F32),
            pltpu.VMEM((D, S), F32),
            pltpu.VMEM((NB, S // 2, 128), I32),
            pltpu.VMEM((H, 24, S), F32),
            pltpu.VMEM((S, D), BF),
            pltpu.SemaphoreType.DMA((NB, 8)),
            pltpu.SemaphoreType.DMA((S // RB,)),
        ],
        compiler_params=pltpu.CompilerParams(vmem_limit_bytes=110 * 2 ** 20),
    )(A_x.reshape(S, D), A_wqkv, A_wo, B_k.reshape(S, D), B_v.reshape(S, D), B_shift_k.T,
      B_ssm_k, B_ssm_D, gate_w, fwd, inv)
    return out.reshape(1, S, D)
```

```python
import numpy as np

import jax
import jax.numpy as jnp
from jax import lax
import jax.experimental.pallas as pl
import jax.experimental.pallas.tpu as pltpu

S = 2048
D = 640
H = 32
DH = D // H
NB = D // 128
L = 128
NC = S // L
PR = 512
TQ = 512
KC = 128
RB = 256
HU = 4

BF = jnp.bfloat16
F32 = jnp.float32
I32 = jnp.int32

QSCALE = float(DH ** -0.5 * np.log2(np.e))
L_MIN = float(2.0 ** -40)
L_MAX = float(2.0 ** 60)


def _dft_tables():
    f = np.concatenate([np.arange(0, L, 2), np.arange(1, L, 2)]).astype(np.float64)
    n = np.arange(L, dtype=np.float64)
    ang = np.pi * (f[:, None] + 0.5) * n[None, :] / L
    fwd = np.concatenate([np.cos(ang), -np.sin(ang)], axis=0)
    inv = fwd.T / L
    return fwd.astype(BF), inv.astype(BF)


def _dot(a, b, ca=1, cb=0):
    return lax.dot_general(a, b, (((ca,), (cb,)), ((), ())), preferred_element_type=F32)


class _Pacer:
    def __init__(self, always):
        self.always = always
        self.link = None

    def dot(self, xs, ys, depth):
        r = None
        for n, (x, y) in enumerate(zip(xs, ys)):
            if n == 0 and self.link is not None and depth is not None:
                y = jnp.where(self.always, y, self.link)
            r = x * y if r is None else r + x * y
            if depth is not None and n == min(depth, len(xs) - 1):
                self.link = r
        return r


class _Lanes:
    def __init__(self, always, width):
        self.always = always
        self.width = width
        self.done = []

    def dot(self, xs, ys, post):
        r = None
        for n, (x, y) in enumerate(zip(xs, ys)):
            if n == 0 and len(self.done) >= self.width:
                y = jnp.where(self.always, y, self.done[-self.width])
            r = x * y if r is None else r + x * y
        self.done.append(post(r))
        return self.done[-1]


def _kernel(x_hbm, w_hbm, wo_hbm, k_hbm, v_hbm, sh_ref, sk_hbm, sd_ref, gw_ref, fwd_ref, inv_ref, zero_ref,
            out_hbm,
            x_v, w_v, wt_v, wo_v, k_v, v_v, sk_v, par_v, kpad, kv_v, uf, kf, yf, b_v,
            qt_v, vt_v, kk_v, ot_v, out_v, sems, xsems, osems):
    def blk(i):
        return pl.ds(i * 128 if isinstance(i, int) else pl.multiple_of(i * 128, 128), 128)

    def sk_copy(i):
        return pltpu.make_async_copy(sk_hbm.at[blk(i), :], sk_v.at[i], sems.at[i, 0])

    def w_copy(i, t):
        return pltpu.make_async_copy(w_hbm.at[:, blk(t * NB + i)], w_v.at[i, t], sems.at[i, 1 + t])

    def k_copy(i):
        return pltpu.make_async_copy(k_hbm.at[:, blk(i)], k_v.at[i], sems.at[i, 4])

    def v_copy(i):
        return pltpu.make_async_copy(v_hbm.at[:, blk(i)], v_v.at[i], sems.at[i, 5])

    def x_copy(r):
        return pltpu.make_async_copy(x_hbm.at[r * PR:(r + 1) * PR, :], x_v.at[r * PR:(r + 1) * PR, :], xsems.at[r])

    def w_copies(i):
        return [w_copy(i, t) for t in range(3)]

    wo_cp = pltpu.make_async_copy(wo_hbm, wo_v, xsems.at[S // PR])
    for cp in [x_copy(0)] + w_copies(0) + w_copies(1):
        cp.start()

    sh = sh_ref[...].astype(F32)
    sd = sd_ref[...].astype(F32).reshape(1, D)
    gw = gw_ref[...].astype(F32).reshape(1, D)
    for i in range(NB):
        cs = slice(i * 128, (i + 1) * 128)
        for j in range(4):
            par_v[i, j] = jnp.broadcast_to(sh[j:j + 1, cs], (8, 128))
        par_v[i, 4] = jnp.broadcast_to(sd[:, cs], (8, 128))
        par_v[i, 5] = jnp.broadcast_to(gw[:, cs], (8, 128))
    kpad[0:8, :] = jnp.zeros((8, 128), F32)

    def run_time_true():
        return fwd_ref[0:16, :].astype(F32)[0:8] < 2.0

    def project(i, r):
        rs = slice(r * PR, (r + 1) * PR)
        kk_v[i, rs, :] = _dot(x_v[rs, :], w_v[i, 1])
        q = _dot(wt_v[i, 0:128, :], x_v[rs, :], 1, 1) * QSCALE
        for t in range(PR // 128):
            qt_v[r * (PR // 128) + t, blk(i), :] = q[:, t * 128:(t + 1) * 128]
        vt_v[blk(i), rs] = _dot(wt_v[i, 128:256, :], x_v[rs, :], 1, 1)

    z = zero_ref[0]

    def spectra(chunks, dst, transposed):
        for c in range(0, NC, 4):
            r = _dot(fwd_ref[...], jnp.concatenate(chunks[c:c + 4], axis=0 if transposed else 1), 1, int(transposed))
            for t in range(4):
                dst[c + t] = r[:, t * 128:(t + 1) * 128]

    def short_conv(i, slot, c, lanes):
        kpad[8 + c * L:8 + (c + 1) * L, :] = k_v[i, c * L:(c + 1) * L, :].astype(F32)
        taps = [par_v[i, j] for j in range(4)]
        vv = v_v[i, c * L:(c + 1) * L, :].astype(F32)
        for a in range(0, L, 8):
            kv_v[(slot if isinstance(slot, int) else z + slot) * NC + c, a:a + 8, :] = lanes.dot(
                [kpad[8 + c * L + a - j:16 + c * L + a - j, :] for j in range(4)], taps, lambda r: r * vv[a:a + 8])

    def chunk_conv(i):
        lanes = _Lanes(run_time_true(), 3)
        yr, yi = [], []
        for g in range(L // 8):
            re = slice(g * 8, (g + 1) * 8)
            im = slice(L + g * 8, L + (g + 1) * 8)
            kr, ki = [kf[z, re, :]], [kf[z, im, :]]
            for d in range(1, NC):
                a, b, pa, pb = kf[z + d, re, :], kf[z + d, im, :], kf[z + d - 1, re, :], kf[z + d - 1, im, :]
                kr.append(a - pb if g < L // 16 else a + pb)
                ki.append(b + pa if g < L // 16 else b - pa)
            ur = [uf[z + d, re, :] for d in range(NC)]
            ui = [uf[z + d, im, :] for d in range(NC)]

            def conv(ks, us, post):
                order = [0, 1, 2, 3, 7, 6, 5, 4, 8, 9, 10, 11, 15, 14, 13, 12]
                if lanes.width == 3:
                    order = range(NC)
                res = {o: lanes.dot(ks[o::-1], us[:o + 1], lambda r: post(o, r)) for o in order}
                return [res[o] for o in range(NC)]

            t1 = conv(kr, [a + b for a, b in zip(ur, ui)], lambda o, r: r)
            yr.append(conv([a + b for a, b in zip(kr, ki)], ui, lambda o, r: t1[o] - r))
            yi.append(conv([b - a for a, b in zip(kr, ki)], ur, lambda o, r: t1[o] + r))
            if 1:
                for o in range(NC):
                    yf[o, re, :] = yr[-1][o]
                    yf[o, im, :] = yi[-1][o]
            short_conv(jnp.minimum(i + 1, NB - 1), i + 1, g, lanes)

    def finish_conv(i):
        for c in range(0, NC, 4):
            y = _dot(inv_ref[...], jnp.concatenate([yf[z + c + t] for t in range(4)], axis=1))
            for t in range(4):
                cs = slice((c + t) * L, (c + t + 1) * L)
                xc = x_v[cs, blk(i)].astype(F32)
                yy = y[:, t * 128:(t + 1) * 128] + kv_v[i * NC + c + t] * jnp.tile(par_v[i, 4], (L // 8, 1))
                b_v[i, cs, :] = xc * yy

    def first_rows(i):
        for cp in w_copies(i):
            cp.wait()
        wt_v[i, 0:128, :] = w_v[i, 0].T
        wt_v[i, 128:256, :] = w_v[i, 2].T
        project(i, 0)

    def first_rows_step(i, carry):
        first_rows(i)
        return carry

    x_copy(0).wait()
    for cp in (w_copies(2) + w_copies(3) + w_copies(4) + [k_copy(0), v_copy(0), sk_copy(0)]
               + [x_copy(r) for r in range(1, S // PR)] + [k_copy(1), v_copy(1)]):
        cp.start()
    lax.fori_loop(0, NB - 1, first_rows_step, 0)
    k_copy(0).wait()
    v_copy(0).wait()
    first_rows(NB - 1)
    lanes0 = _Lanes(run_time_true(), 2)
    for c in range(NC):
        short_conv(0, 0, c, lanes0)
    for i in range(1, NB):
        for cp in [sk_copy(i)] + ([k_copy(i + 1), v_copy(i + 1)] if i + 1 < NB else [wo_cp]):
            cp.start()

    def block_step(i, carry):
        sk_copy(i).wait()
        spectra([sk_v[i, :, c * L:(c + 1) * L] for c in range(NC)], kf, True)
        spectra([kv_v[i * NC + c] for c in range(NC)], uf, False)

        @pl.when(i == 0)
        def _():
            for r in range(1, S // PR):
                x_copy(r).wait()

        @pl.when(i + 1 < NB)
        def _():
            k_copy(i + 1).wait()
            v_copy(i + 1).wait()

        for r in range(1, S // PR):
            project(i, r)
        chunk_conv(i)
        finish_conv(i)
        return carry

    lax.fori_loop(0, NB, block_step, 0)

    sub = lax.broadcasted_iota(I32, (8, 128), 0)
    lane = lax.broadcasted_iota(I32, (8, 128), 1)

    def head_views(h, odd):
        r0 = pl.multiple_of(h * DH - 4 * odd, 8)
        b0 = r0 // 128
        b1 = jnp.minimum(b0 + 1, NB - 1)
        l0 = r0 - b0 * 128

        def fill(x, val):
            n = x.shape[1] // 128
            if odd:
                return jnp.concatenate([jnp.where(jnp.tile(sub >= 4, (1, n)), x[0:8], val), x[8:24]], axis=0)
            return jnp.concatenate([x[0:16], jnp.where(jnp.tile(sub < 4, (1, n)), x[16:24], val)], axis=0)

        def keys(a, n):
            kk = jnp.where(jnp.tile(lane >= l0, (n // 8, 1)), kk_v[b0, a:a + n, :], kk_v[b1, a:a + n, :])
            return pltpu.roll(kk, (128 - l0) & 127, 1)

        def queries(t0, n):
            q = fill(jnp.concatenate([qt_v[t0 + t, pl.ds(r0, 24), :] for t in range(n)], axis=1), 0.0)
            return jnp.concatenate([q, jnp.zeros((8, n * 128), F32)], axis=0).astype(BF)

        def values(a, n):
            return fill(vt_v[pl.ds(r0, 24), a:a + n], 1.0)

        return keys, queries, values

    nq, nk = S // TQ, S // KC
    NVP = [int(ch) for ch in "2"]
    NV0 = [int(ch) for ch in "0"]

    def heads_fast(hh, carry):
        lo, hi = carry
        pacer = _Pacer(run_time_true())
        views = [head_views(hh * HU + u, u & 1) for u in range(HU)]
        steps = [(u, c, j) for u in range(HU) for c in range(nk) for j in range(nq)]
        acc, p_prev = {}, None
        for t in range(len(steps) + 1):
            if t < len(steps):
                u, c, j = steps[t]
                g = u * nk + c
                nv = NV0[g] if g < len(NV0) else NVP[g % len(NVP)]
                if c == 0 and j == 0:
                    qs = [views[u][1](jj * 4, 4) for jj in range(nq)]
                    qb = [[jnp.broadcast_to(qt_v[tile, pl.ds((hh * HU + u) * DH + d, 1), :], (8, 128))
                           for d in range(DH)] for tile in range(S // 128)]
                if j == 0:
                    kc = views[u][0](c * KC, KC)
                    km = jnp.concatenate([kc[r * 8:(r + 1) * 8] for r in reversed(range(nv, KC // 8))], axis=0)
                    km = km[:, :32].astype(F32 if nv % 2 else BF)
                    f0 = 4 * (u & 1)
                    kb = [[jnp.broadcast_to(kc[a * 8:(a + 1) * 8, f0 + d:f0 + d + 1], (8, 128))
                           for d in range(DH)] for a in range(nv)]
                s = _dot(km, qs[j])
                x = [[pacer.dot(kb[a], qb[j * 4 + b], 6) for a in range(nv)] for b in range(4)]
                s = ([jnp.concatenate([x[b][a] for b in range(4)], axis=1) for a in range(nv)]
                     + [s[r * 8:(r + 1) * 8] for r in reversed(range(KC // 8 - nv))])
                p_new = jnp.exp2(jnp.concatenate(s, axis=0))
            if t >= 1:
                u, c, j = steps[t - 1]
                if j == 0:
                    vc = views[u][2](c * KC, KC)
                r = _dot(vc, p_prev)
                o = acc[j] = r if c == 0 else acc[j] + r
                if c == 0 or c == nk - 1:
                    ot_v[hh * HU + u, :, j * TQ:(j + 1) * TQ] = o
                if c == nk - 1:
                    for b in range(4):
                        ob = o[:, b * 128:(b + 1) * 128]
                        den = jnp.where(sub < 4, ob[0:8], 1.0) if u & 1 else jnp.where(sub >= 4, ob[16:24], 1.0)
                        lo = jnp.minimum(lo, den)
                        ob = jnp.abs(ob)
                        hi = jnp.maximum(hi, jnp.maximum(jnp.maximum(ob[0:8], ob[8:16]), ob[16:24]))
            p_prev = p_new
        return lo, hi

    lo, hi = jnp.ones((8, 128), F32), jnp.ones((8, 128), F32)
    if not 0:
        lo, hi = lax.fori_loop(0, H // HU, heads_fast, (lo, hi))

    safe = (lo >= L_MIN) & (hi <= L_MAX)
    n_bad = jnp.sum(jnp.where(safe, 0.0, 1.0))

    @pl.when(n_bad > 0.0)
    def _():
        def pair_exact(t, carry):
            tile = t % (S // 128)
            for odd in range(2):
                h = 2 * (t // (S // 128)) + odd
                keys, queries, values = head_views(h, odd)
                s = _dot(keys(0, S)[:, :32].astype(BF), queries(tile, 1))
                p = jnp.exp2(s - jnp.max(s, axis=0, keepdims=True))
                ot_v[h, :, blk(tile)] = _dot(values(0, S), p)
            return carry

        lax.fori_loop(0, (H // 2) * (S // 128), pair_exact, 0)

    wo_cp.wait()
    low4 = lax.broadcasted_iota(I32, (8, RB), 0) < 4
    OU = 4

    def rows(r):
        return pl.ds(r * RB if isinstance(r, int) else pl.multiple_of(r * RB, RB), RB)

    def out_copy(r):
        return pltpu.make_async_copy(out_v.at[r], out_hbm.at[rows(r), :], osems.at[r])

    def out_blocks(n, carry):
        for r in [n * OU + t for t in range(OU)]:
            rs = rows(r)
            parts = []
            for p in range(H // 2):
                e, o = ot_v[2 * p, :, rs], ot_v[2 * p + 1, :, rs]
                inv_l = 1.0 / jnp.where(low4, o[0:8], e[16:24])
                e = e * jnp.broadcast_to(inv_l[7:8], (24, RB))
                o = o * jnp.broadcast_to(inv_l[0:1], (24, RB))
                parts += [e[0:16], jnp.where(low4, e[16:24], o[0:8]), o[8:24]]
            a = _dot(jnp.concatenate(parts, axis=0).astype(BF), wo_v[...], 0, 0)
            gx = [x_v[rs, blk(t)].astype(F32) * jnp.tile(par_v[t, 5], (RB // 8, 1)) for t in range(NB)]
            g = jax.nn.sigmoid(jnp.sum(sum(gx[1:], gx[0]), axis=1, keepdims=True))
            b = jnp.concatenate([b_v[t, rs, :] for t in range(NB)], axis=1)
            out_v[r] = (g * a + (1.0 - g) * b).astype(BF)
            out_copy(r).start()
        return carry

    if OU == S // RB:
        out_blocks(0, 0)
    else:
        lax.fori_loop(0, S // RB // OU, out_blocks, 0)
    for r in range(S // RB):
        out_copy(r).wait()


@jax.jit
def pallas_gated_mix__mha_block__ssm_conv_h3__prompt_kernel(
    A_x: jax.Array,
    A_wqkv: jax.Array,
    A_wo: jax.Array,
    B_q: jax.Array,
    B_k: jax.Array,
    B_v: jax.Array,
    B_shift_k: jax.Array,
    B_ssm_k: jax.Array,
    B_ssm_D: jax.Array,
    gate_w: jax.Array,
):
    del B_q
    fwd, inv = _dft_tables()
    hbm = pl.BlockSpec(memory_space=pl.ANY)
    vmem = pl.BlockSpec(memory_space=pltpu.VMEM)
    out = pl.pallas_call(
        _kernel,
        in_specs=[hbm, hbm, hbm, hbm, hbm, vmem, hbm, vmem, vmem, vmem, vmem, pl.BlockSpec(memory_space=pltpu.SMEM)],
        out_specs=hbm,
        out_shape=jax.ShapeDtypeStruct((S, D), BF),
        scratch_shapes=[
            pltpu.VMEM((S, D), BF),
            pltpu.VMEM((NB, 3, D, 128), BF),
            pltpu.VMEM((NB, 256, D), BF),
            pltpu.VMEM((D, D), BF),
            pltpu.VMEM((NB, S, 128), BF),
            pltpu.VMEM((NB, S, 128), BF),
            pltpu.VMEM((NB, 128, S), BF),
            pltpu.VMEM((NB, 8, 8, 128), F32),
            pltpu.VMEM((S + 32, 128), F32),
            pltpu.VMEM(((NB + 1) * NC, L, 128), F32),
            pltpu.VMEM((NC, 2 * L, 128), F32),
            pltpu.VMEM((NC, 2 * L, 128), F32),
            pltpu.VMEM((NC, 2 * L, 128), F32),
            pltpu.VMEM((NB, S, 128), F32),
            pltpu.VMEM((S // 128, D, 128), F32),
            pltpu.VMEM((D, S), F32),
            pltpu.VMEM((NB, S, 128), F32),
            pltpu.VMEM((H, 24, S), F32),
            pltpu.VMEM((S // RB, RB, D), BF),
            pltpu.SemaphoreType.DMA((NB, 6)),
            pltpu.SemaphoreType.DMA((S // PR + 1,)),
            pltpu.SemaphoreType.DMA((S // RB,)),
        ],
        compiler_params=pltpu.CompilerParams(vmem_limit_bytes=110 * 2 ** 20),
    )(A_x.reshape(S, D), A_wqkv, A_wo, B_k.reshape(S, D), B_v.reshape(S, D), B_shift_k.T,
      B_ssm_k, B_ssm_D, gate_w, fwd, inv, np.zeros((1,), np.int32))
    return out.reshape(1, S, D)
```

```python
import functools

import numpy as np

import jax
import jax.numpy as jnp
from jax import lax
import jax.experimental.pallas as pl
import jax.experimental.pallas.tpu as pltpu

S = 2048
D = 640
H = 32
DH = D // H
NB = D // 128
L = 128
NC = S // L
PR = 512
TQ = 512
KC = 128
G = 2
RB = 256
HU = 4
TP = 9

BF = jnp.bfloat16
F32 = jnp.float32
I32 = jnp.int32

QSCALE = float(DH ** -0.5 * np.log2(np.e))
FULL = 127 * 32
UNIT = 512.0 / FULL ** 2
TINY = 1e-30
TERM_MAX = 8.0
SUM_MIN = float(2.0 ** -40)
SUM_MAX = float(2.0 ** 60)


def _dft_tables():
    s, k, a = np.meshgrid(np.arange(2), np.arange(8), np.arange(8), indexing="ij")
    ang = np.pi * (2 * (s + 2 * a + 16 * k) + 0.5).reshape(-1, 1) * np.arange(L) / L
    dense = np.concatenate([np.cos(ang), -np.sin(ang)], axis=0)
    ang = np.pi * (2 * (s + 2 * a) + 0.5) * k / L
    twiddle = np.stack([np.cos(ang), np.sin(ang)], axis=2)[..., None] * np.ones(128)
    return dense.astype(BF), twiddle.astype(np.float32)


_THETA = np.pi * (2 * np.arange(2)[:, None] + 0.5) * np.arange(16) / 16


def _dft8(x, sign):
    def add(a, b):
        return a[0] + b[0], a[1] + b[1]

    def sub(a, b):
        return a[0] - b[0], a[1] - b[1]

    def rot(a, b):
        p, m = (a[0] - b[1], a[1] + b[0]), (a[0] + b[1], a[1] - b[0])
        return (p, m) if sign > 0 else (m, p)

    def dft4(a, b, c, d):
        s0, s1 = add(a, c), add(b, d)
        o1, o3 = rot(sub(a, c), sub(b, d))
        return add(s0, s1), o1, sub(s0, s1), o3

    def eighth(a):
        r = float(np.sqrt(0.5))
        return ((a[0] - a[1]) * r, (a[0] + a[1]) * r) if sign > 0 else ((a[0] + a[1]) * r, (a[1] - a[0]) * r)

    e, o = dft4(*x[0::2]), dft4(*x[1::2])
    t1 = eighth(o[1])
    x2, x6 = rot(e[2], o[2])
    x3, x7 = rot(e[3], eighth(o[3]))
    return [add(e[0], o[0]), add(e[1], t1), x2, x3, sub(e[0], o[0]), sub(e[1], t1), x6, x7]


def _limbs(x, is_key):
    n = pltpu.bitcast(x + float(1.5 * 2 ** 23), I32)
    word = (((n + 8) >> 5) & 0xFF) | (((n + 24) << 3) & 0xFF00)
    if is_key:
        word = word | (((n << 28) >> 12) & 0xFF0000) | (((n + 256) >> 9) << 24)
    else:
        word = word | (((n + 256) << 7) & 0xFF0000) | ((n << 28) >> 4)
    return word


def _dot(a, b, ca=1, cb=0, out=F32):
    return lax.dot_general(a, b, (((ca,), (cb,)), ((), ())), preferred_element_type=out)


def _sum_of_products(xs, ys):
    r = xs[0] * ys[0]
    for x, y in zip(xs[1:], ys[1:]):
        r = r + x * y
    return r


def _kernel(x_hbm, w_hbm, wo_hbm, k_hbm, v_hbm, sh_hbm, sk_hbm, sd_hbm, gw_hbm, fwd_hbm, tw_hbm, zero_ref,
            out_hbm,
            x_v, w_v, wt_v, wo_v, k_v, v_v, sk_v, par_v, kpad, uf, kf, yf, y_v, g_v,
            qt_v, kt_v, vt_v, ot_v, out_v, ktop_v, key_v, qry_v, tr_v, tw_v, fwd_v, inv_v, sh_v, sd_v, gw_v,
            sems, xsems, osems, psems):
    z = zero_ref[0]

    def blk(i):
        return pl.ds(i * 128 if isinstance(i, int) else pl.multiple_of(i * 128, 128), 128)

    def after(x, dep, bound=2.0):
        return jnp.where(tw_v[0, 0, 0] < bound, x, dep)

    def w_copies(i):
        return [pltpu.make_async_copy(w_hbm.at[:, blk(t * NB + i)], w_v.at[i, t], sems.at[i, t]) for t in range(3)]

    def quarter(r):
        return pl.ds(r * PR if isinstance(r, int) else pl.multiple_of(r * PR, PR), PR)

    def conv_copies(i):
        last = blk(NB - 1)
        pairs = [(sk_hbm.at[blk(i), :], sk_v.at[i, :, 0:S]), (sk_hbm.at[last, quarter(i)], sk_v.at[i, :, S:S + PR]),
                 (k_hbm.at[:, blk(i)], k_v.at[i, 0:S]), (k_hbm.at[quarter(i), last], k_v.at[i, S:S + PR]),
                 (v_hbm.at[:, blk(i)], v_v.at[i, 0:S]), (v_hbm.at[quarter(i), last], v_v.at[i, S:S + PR])]
        return [pltpu.make_async_copy(src, dst, sems.at[i, 3 + n]) for n, (src, dst) in enumerate(pairs)]

    def x_copy(r):
        return pltpu.make_async_copy(x_hbm.at[quarter(r), :], x_v.at[quarter(r), :], xsems.at[r])

    wo_copy = pltpu.make_async_copy(wo_hbm, wo_v, xsems.at[S // PR])
    small_copies = [pltpu.make_async_copy(src, dst, psems.at[n]) for n, (src, dst) in enumerate(
        [(sh_hbm, sh_v), (sd_hbm, sd_v), (gw_hbm, gw_v), (fwd_hbm, fwd_v), (tw_hbm, tw_v)])]

    def start(copies):
        for cp in copies:
            cp.start()

    def wait(copies):
        for cp in copies:
            cp.wait()

    def spread_parameters():
        sh = sh_v[...].astype(F32)
        sd = sd_v[...].astype(F32).reshape(1, D)
        gw = gw_v[...].astype(F32).reshape(1, D)
        for i in range(NB):
            cs = slice(i * 128, (i + 1) * 128)
            for j in range(4):
                par_v[i, j] = jnp.broadcast_to(sh[j:j + 1, cs], (8, 128))
            par_v[i, 4] = jnp.broadcast_to(sd[:, cs], (8, 128))
            par_v[i, 5] = jnp.broadcast_to(gw[:, cs], (8, 128))
        kpad[0:8, :] = jnp.zeros((8, 128), F32)
        kpad[S + PR + 8:S + PR + 16, :] = jnp.zeros((8, 128), F32)
        inv_v[...] = (fwd_v[...].astype(F32).T * (1.0 / L)).astype(BF)

    def short_conv(i, c, dot):
        r0 = 8 + c * L + (8 if c >= NC else 0)
        if c == NC:
            kpad[r0 - 8:r0, :] = kpad[r0 + PR - 8:r0 + PR, :]
        kpad[r0:r0 + L, :] = k_v[i, c * L:(c + 1) * L, :].astype(F32)
        taps = [par_v[i if c < NC else NB - 1, j] for j in range(4)]
        vv = v_v[i, c * L:(c + 1) * L, :].astype(F32)
        return [dot([kpad[r0 + a - j:r0 + a - j + 8, :] for j in range(4)], taps,
                    lambda r: r * vv[a:a + 8]) for a in range(0, L, 8)]

    def transposed(slot, tiles):
        for n, v in enumerate(tiles):
            tr_v[(slot * 8 + n) * TP:(slot * 8 + n) * TP + 8, :] = v
        return [tr_v[pl.ds(slot * 8 * TP + n, 8, stride=TP), :] for n in range(8)]

    def forward_fft(x, tile):
        for s in range(2):
            co, si = np.cos(_THETA[s]), -np.sin(_THETA[s])
            a = [(x[0] + x[8] * float(co[8]), x[8] * float(si[8]))]
            a += [(x[m] * float(co[m]) + x[m + 8] * float(co[m + 8]),
                   x[m] * float(si[m]) + x[m + 8] * float(si[m + 8])) for m in range(1, 8)]
            a = _dft8(a, -1)
            b = list(zip(transposed(2 * s, [v[0] for v in a]), transposed(2 * s + 1, [v[1] for v in a])))
            for n in range(1, 8):
                p, q = tw_v[s, n, 0], tw_v[s, n, 1]
                b[n] = (b[n][0] * p + b[n][1] * q, b[n][1] * p - b[n][0] * q)
            for k, (re, im) in enumerate(_dft8(b, -1)):
                uf[tile, 64 * s + 8 * k:64 * s + 8 * k + 8, :] = re
                uf[tile, L + 64 * s + 8 * k:L + 64 * s + 8 * k + 8, :] = im

    def chunk_conv(i, g0, g, dot):
        re = pl.ds(pl.multiple_of(g0 * 8, 32) + g * 8, 8)
        im = pl.ds(pl.multiple_of(g0 * 8, 32) + g * 8 + L, 8)
        t0 = i * NC
        kr, ki = [kf[t0, re, :] + par_v[i, 4]], [kf[t0, im, :]]
        for d in range(1, NC):
            kr.append(kf[t0 + d, re, :] - kf[t0 + d - 1, im, :])
            ki.append(kf[t0 + d, im, :] + kf[t0 + d - 1, re, :])
        ur = [uf[t0 + d, re, :] for d in range(NC)]
        ui = [uf[t0 + d, im, :] for d in range(NC)]
        us, t1 = [a + b for a, b in zip(ur, ui)], []
        for o in range(NC):
            t1.append(dot(kr[o::-1], us[:o + 1], lambda r: r))
            yield t1[o]
        ks = [a + b for a, b in zip(kr, ki)]
        for o in range(NC):
            y = yf[t0 + o, re, :] = dot(ks[o::-1], ui[:o + 1], lambda r: t1[o] - r)
            yield y
        ks = [b - a for a, b in zip(kr, ki)]
        for o in range(NC):
            y = yf[t0 + o, im, :] = dot(ks[o::-1], ur[:o + 1], lambda r: t1[o] + r)
            yield y

    def inverse_fft(tile):
        halves = []
        for s in range(2):
            b = _dft8([(yf[tile, 64 * s + 8 * k:64 * s + 8 * k + 8, :],
                        yf[tile, L + 64 * s + 8 * k:L + 64 * s + 8 * k + 8, :]) for k in range(8)], 1)
            for n in (0, 4, 2, 6, 1, 5, 3, 7):
                if n:
                    p, q = tw_v[s, n, 0], tw_v[s, n, 1]
                    b[n] = (b[n][0] * p - b[n][1] * q, b[n][0] * q + b[n][1] * p)
                yield from b[n]
            halves.append(_dft8(list(zip(transposed(2 * s, [v[0] for v in b]),
                                         transposed(2 * s + 1, [v[1] for v in b]))), 1))
        for m in (0, 8, 4, 12, 2, 10, 6, 14, 1, 9, 5, 13, 3, 11, 7, 15):
            y = None
            for s in range(2):
                t = halves[s][m % 8][0] * float(np.cos(_THETA[s, m]) / L)
                if m:
                    t = t - halves[s][m % 8][1] * float(np.sin(_THETA[s, m]) / L)
                y = t if y is None else y + t
            y_v[tile, 8 * m:8 * m + 8, :] = y
            yield y

    def gate_terms(r0, r):
        rs = pl.ds(pl.multiple_of(r0, 128) + r, 32)
        g = _sum_of_products([x_v[rs, blk(t)].astype(F32) for t in range(NB)],
                             [jnp.tile(par_v[t, 5], (4, 1)) for t in range(NB)])
        g_v[rs, :] = g
        for a in range(0, 32, 8):
            yield g[a:a + 8]

    def transpose_weights(i):
        for t in range(3):
            wt_v[t] = w_v[i, t].T

    def project(i, r, top):
        qt_v[blk(i), quarter(r)] = _dot(wt_v[0], x_v[quarter(r), :], 1, 1)
        k = kt_v[blk(i), quarter(r)] = _dot(wt_v[1], x_v[quarter(r), :], 1, 1)
        vt_v[blk(i), quarter(r)] = _dot(wt_v[2], x_v[quarter(r), :], 1, 1)
        return functools.reduce(jnp.maximum, [jnp.abs(k[:, a:a + 128]) for a in range(0, PR, 128)], top)

    def set_key_range(i, top):
        ktop_v[blk(i), :] = jnp.broadcast_to(jnp.max(top, axis=1, keepdims=True), (128, 128))

    def first_block(r, carry):
        wait([x_copy(r)])
        for n, copies in enumerate([[x_copy(2), x_copy(3)] + small_copies, conv_copies(0) + w_copies(1)]):
            pl.when(r == n)(functools.partial(start, copies))
        ktop_v[0:128, :] = project(0, r, ktop_v[0:128, :])
        return carry

    def feature_block(i, carry):
        wait(conv_copies(i) + w_copies(i + 1))

        def tile(c):
            return i * NC + c if c < NC else (NB - 1) * NC + i * (PR // L) + c - NC

        for c in range(0, NC + PR // L, 4):
            r = _dot(fwd_v[...], jnp.concatenate([sk_v[i, :, blk(c + t)] for t in range(4)], axis=0), 1, 1)
            for t in range(4):
                kf[tile(c + t)] = r[:, t * 128:(t + 1) * 128]
        transpose_weights(i + 1)
        top = TINY
        for r in range(S // PR):
            top = project(i + 1, r, top)
        set_key_range(i + 1, top)

        done = []

        def paced(xs, ys, post):
            if len(done) >= 4:
                ys = [after(ys[0], done[-4])] + ys[1:]
            done.append(post(_sum_of_products(xs, ys)))
            return done[-1]

        for c in range(NC + PR // L):
            forward_fft(short_conv(i, c, paced), tile(c))
        for g in range(4):
            for _ in chunk_conv(z, i * 4, g, paced):
                pass
        tr_v[0:8, :] = _dot(done[-1] + done[-2] + done[-3], fwd_v[0:128, :])

        @pl.when(i + 3 < NB)
        def _():
            start(conv_copies(i + 2) + w_copies(i + 3))

        return carry

    sub = lax.broadcasted_iota(I32, (8, 128), 0)
    nq, nk = S // TQ, S // KC

    def head_rows(first, u):
        return pl.ds(pl.multiple_of(first * DH, 8) + (u * DH - 4 * (u & 1)), 24)

    def own(x, odd, other):
        n = x.shape[1] // 128
        if odd:
            return jnp.concatenate([jnp.where(jnp.tile(sub >= 4, (1, n)), x[0:8], other), x[8:24]], axis=0)
        return jnp.concatenate([x[0:16], jnp.where(jnp.tile(sub < 4, (1, n)), x[16:24], other)], axis=0)

    def key_limbs(rows, gain, c):
        words, out = [], []
        for n in range(c, c + G):
            w = _limbs(kt_v[rows, blk(n)] * gain, True)
            words += [w[r:r + 8] for r in (0, 8, 16)]
            w = pltpu.bitcast(jnp.concatenate([w, jnp.zeros((8, KC), I32)], axis=0), jnp.int8)
            w = pltpu.bitcast(w.T, I32)
            out += [w[r:r + 8] for r in (24, 16, 8, 0)]
        return words, out

    def query_limbs(rows, odd, tile):
        q = qt_v[rows, blk(tile)] * own(ktop_v[rows, :] * QSCALE, odd, 0.0)
        a = jnp.abs(q)
        q_top = jnp.max(jnp.maximum(jnp.maximum(a[0:8], a[8:16]), a[16:24]), axis=0, keepdims=True)
        q_top = jnp.broadcast_to(jnp.maximum(q_top, TINY), (8, 128))
        inv = pl.reciprocal(q_top, approx=True)
        inv = inv * (2.0 * FULL - FULL * q_top * inv)
        return _limbs(q * jnp.tile(inv, (3, 1)), False), after(q_top * UNIT, q_top)

    def stage(keys, queries):
        key_v[...] = jnp.concatenate(keys, axis=0)
        for tile, (limbs, unit) in enumerate(queries):
            qry_v[tile, 0:24] = limbs
            qry_v[tile, 24:32] = pltpu.bitcast(unit, I32)

    def heads_fast(hh, carry):
        lo, hi, top = carry
        n_side = (NB - 1) * NC * HU // H

        def side_work():
            for n in range(n_side):
                yield from inverse_fft(z + hh * n_side + n)
                yield from gate_terms(hh * n_side * 32, n * 32)
                yield from chunk_conv(1 + hh * n_side // NC, hh * n_side % NC, n,
                                      lambda xs, ys, post: post(_sum_of_products(xs, ys)))

        work = side_work()
        acc, values, pending = {}, {}, []

        def weighted_values(u, c, j, p):
            nonlocal lo, hi
            if j == 0:
                values[c] = own(vt_v[head_rows(hh * HU, u), blk(c)], u & 1, 1.0)
            r = _dot(values[c], p)
            o = acc[j] = r if c == 0 else acc[j] + r
            if c == G - 1 or c == nk - 1:
                ot_v[hh * HU + u, :, j * TQ:(j + 1) * TQ] = o
            if c == nk - 1:
                for b in range(4):
                    ob = o[:, b * 128:(b + 1) * 128]
                    den = jnp.where(sub < 4, ob[0:8], 1.0) if u & 1 else jnp.where(sub >= 4, ob[16:24], 1.0)
                    lo = jnp.minimum(lo, den)
                    ob = jnp.abs(ob)
                    hi = jnp.maximum(hi, jnp.maximum(jnp.maximum(ob[0:8], ob[8:16]), ob[16:24]))

        slot = 0
        rows = head_rows(hh * HU, 0)
        gain = FULL / ktop_v[rows, :]
        next_keys = [key_v[...]]
        next_queries = [(qry_v[t, 0:24], pltpu.bitcast(qry_v[t, 24:32], F32)) for t in range(S // 128)]
        for u, c, j in [(u, c, j) for u in range(HU) for c in range(0, nk, G) for j in range(nq)]:
            following = head_rows(hh * HU, u + 1) if u + 1 < HU else head_rows(jnp.minimum(hh + 1, H // HU - 1) * HU, 0)
            if c == 0 and j == 0:
                queries, next_queries = next_queries, []
                top = functools.reduce(jnp.maximum, [unit for _, unit in queries], top)
            if j == 0:
                keys = pltpu.bitcast(jnp.concatenate(next_keys, axis=0), jnp.int8)[:, :96]
                if c + G == nk:
                    rows, gain = following, FULL / ktop_v[following, :]
                words, next_keys = key_limbs(rows, gain, (c + G) % nk)
            early = [words[0:3], words[3:6], [], next_keys[0::4]][j]
            if j >= 2:
                next_queries.append(query_limbs(following, (u + 1) & 1, len(next_queries)))
                limbs, unit = next_queries[-1]
                early = [unit] + [limbs[r:r + 8] for r in (0, 8, 16)] + early
            limbs = jnp.concatenate([q[0] for q in queries[4 * j:4 * j + 4]], axis=1)
            s = _dot(keys, pltpu.bitcast(limbs, jnp.int8), out=I32).astype(F32)
            slot += 1
            side = [next(work, None) for _ in range(6 + (slot % 5 < 2))] if slot > 1 else []
            side = [pltpu.bitcast(d, I32) for d in side if d is not None]
            early = [pltpu.bitcast(d, I32) for d in early]
            deps = {}
            for items, where, b in ((side, (0, 0, 1, 1, 2, 3, 6), 0), (early, (0, 0, 1, 2, 2, 2), 2)):
                for d, r in zip(items, where):
                    deps.setdefault((r, b), []).append(d)
            for n in range(G):
                parts = []
                for r in range(4 * n, 4 * n + 4):
                    units = [q[1] for q in queries[4 * j:4 * j + 4]]
                    for b in range(4):
                        if (r, b) in deps:
                            units[b] = after(units[b], pltpu.bitcast(functools.reduce(jnp.bitwise_or, deps[r, b]), F32), 3.0)
                    parts.append(s[r * 32:(r + 1) * 32] * jnp.tile(jnp.concatenate(units, axis=1), (4, 1)))
                p = jnp.exp2(jnp.concatenate(parts[::-1], axis=0))
                pending.append((u, c + n, j, p))
            while len(pending) > G:
                weighted_values(*pending.pop(0))
        for item in pending:
            weighted_values(*item)
        assert next(work, None) is None
        stage(next_keys, next_queries)
        return lo, hi, top

    start(w_copies(0) + [x_copy(0)])
    ktop_v[0:128, :] = jnp.full((128, 128), TINY, F32)
    wait(w_copies(0))
    start([x_copy(1)])
    transpose_weights(0)
    lax.fori_loop(0, S // PR, first_block, 0)
    wait(small_copies)
    spread_parameters()
    set_key_range(0, ktop_v[0:128, :])
    stage(key_limbs(pl.ds(0, 24), FULL / ktop_v[0:24, :], 0)[1],
          [query_limbs(pl.ds(0, 24), 0, t) for t in range(S // 128)])
    start(conv_copies(1) + w_copies(2))
    lax.fori_loop(0, NB - 1, feature_block, 0)
    start([wo_copy])
    ones = jnp.ones((8, 128), F32)
    lo, hi, top = lax.fori_loop(0, H // HU, heads_fast, (ones, ones, jnp.zeros((8, 128), F32)))

    safe = (lo >= SUM_MIN) & (hi <= SUM_MAX) & (top <= TERM_MAX * UNIT)

    @pl.when(jnp.sum(jnp.where(safe, 0.0, 1.0)) > 0.0)
    def _():
        def pair_exact(t, carry):
            first = 2 * (t // nq)
            qs = pl.ds(pl.multiple_of(t % nq * TQ, TQ), TQ)
            for odd in range(2):
                rows = head_rows(first, odd)
                q = own(qt_v[rows, qs] * QSCALE, odd, 0.0)

                def chunk(c, state):
                    m, o = state
                    s = _dot(kt_v[rows, blk(c)], q, 0, 0)
                    m_new = jnp.maximum(m, jnp.max(s, axis=0, keepdims=True))
                    pv = _dot(own(vt_v[rows, blk(c)], odd, 1.0), jnp.exp2(s - m_new))
                    return m_new, o * jnp.exp2(m - m_new) + pv

                init = jnp.full((1, TQ), -jnp.inf, F32), jnp.zeros((24, TQ), F32)
                ot_v[first + odd, :, qs] = lax.fori_loop(0, nk, chunk, init)[1]
            return carry

        lax.fori_loop(0, (H // 2) * nq, pair_exact, 0)

    wait([wo_copy])
    for t0 in range((NB - 1) * NC, NB * NC, 4):
        y = _dot(inv_v[...], jnp.concatenate([yf[t0 + t] for t in range(4)], axis=1))
        for t in range(4):
            y_v[t0 + t] = y[:, t * 128:(t + 1) * 128]
    low4 = lax.broadcasted_iota(I32, (8, RB), 0) < 4
    out_copies = []
    for r in range(S // RB):
        rs = slice(r * RB, (r + 1) * RB)
        parts = []
        for p in range(H // 2):
            e, o = ot_v[2 * p, :, rs], ot_v[2 * p + 1, :, rs]
            den = jnp.where(low4, o[0:8], e[16:24])
            inv = pl.reciprocal(den, approx=True)
            inv = inv * (2.0 - den * inv)
            e = e * jnp.broadcast_to(inv[7:8], (24, RB))
            o = o * jnp.broadcast_to(inv[0:1], (24, RB))
            parts += [e[0:16], jnp.where(low4, e[16:24], o[0:8]), o[8:24]]
        a = _dot(jnp.concatenate(parts, axis=0).astype(BF), wo_v[...], 0, 0)
        g = jax.nn.sigmoid(jnp.sum(g_v[rs, :], axis=1, keepdims=True))
        mixed = []
        for t in range(NB):
            y = y_v[t * NC + r * (RB // L):t * NC + (r + 1) * (RB // L)].reshape(RB, 128)
            b = x_v[rs, blk(t)].astype(F32) * y
            mixed.append(b + g * (a[:, t * 128:(t + 1) * 128] - b))
        out_v[r] = jnp.concatenate(mixed, axis=1).astype(BF)
        out_copies.append(pltpu.make_async_copy(out_v.at[r], out_hbm.at[rs, :], osems.at[r]))
        out_copies[-1].start()
    wait(out_copies)


@jax.jit
def pallas_gated_mix__mha_block__ssm_conv_h3__prompt_kernel(
    A_x: jax.Array,
    A_wqkv: jax.Array,
    A_wo: jax.Array,
    B_q: jax.Array,
    B_k: jax.Array,
    B_v: jax.Array,
    B_shift_k: jax.Array,
    B_ssm_k: jax.Array,
    B_ssm_D: jax.Array,
    gate_w: jax.Array,
):
    del B_q
    dense, twiddle = _dft_tables()
    hbm = pl.BlockSpec(memory_space=pl.ANY)
    out = pl.pallas_call(
        _kernel,
        in_specs=[hbm] * 11 + [pl.BlockSpec(memory_space=pltpu.SMEM)],
        out_specs=hbm,
        out_shape=jax.ShapeDtypeStruct((S, D), BF),
        scratch_shapes=[
            pltpu.VMEM((S, D), BF),
            pltpu.VMEM((NB, 3, D, 128), BF),
            pltpu.VMEM((3, 128, D), BF),
            pltpu.VMEM((D, D), BF),
            pltpu.VMEM((NB - 1, S + PR, 128), BF),
            pltpu.VMEM((NB - 1, S + PR, 128), BF),
            pltpu.VMEM((NB - 1, 128, S + PR), BF),
            pltpu.VMEM((NB, 8, 8, 128), F32),
            pltpu.VMEM((S + PR + 32, 128), F32),
            pltpu.VMEM((NB * NC, 2 * L, 128), F32),
            pltpu.VMEM((NB * NC, 2 * L, 128), F32),
            pltpu.VMEM((NB * NC, 2 * L, 128), F32),
            pltpu.VMEM((NB * NC, L, 128), F32),
            pltpu.VMEM((S, 128), F32),
            pltpu.VMEM((D, S), F32),
            pltpu.VMEM((D, S), F32),
            pltpu.VMEM((D, S), F32),
            pltpu.VMEM((H, 24, S), F32),
            pltpu.VMEM((S // RB, RB, D), BF),
            pltpu.VMEM((D, 128), F32),
            pltpu.VMEM((64, 128), I32),
            pltpu.VMEM((S // 128, 32, 128), I32),
            pltpu.VMEM((32 * TP + 32, 128), F32),
            pltpu.VMEM((2, 8, 2, 8, 128), F32),
            pltpu.VMEM((2 * L, L), BF),
            pltpu.VMEM((L, 2 * L), BF),
            pltpu.VMEM((4, D), BF),
            pltpu.VMEM((D,), BF),
            pltpu.VMEM((D,), BF),
            pltpu.SemaphoreType.DMA((NB, 9)),
            pltpu.SemaphoreType.DMA((S // PR + 1,)),
            pltpu.SemaphoreType.DMA((S // RB,)),
            pltpu.SemaphoreType.DMA((5,)),
        ],
        compiler_params=pltpu.CompilerParams(vmem_limit_bytes=110 * 2 ** 20),
    )(A_x.reshape(S, D), A_wqkv, A_wo, B_k.reshape(S, D), B_v.reshape(S, D), B_shift_k.T,
      B_ssm_k, B_ssm_D, gate_w, dense, twiddle, np.zeros((1,), np.int32))
    return out.reshape(1, S, D)
```
